```python
import os as _os
_os.environ.setdefault("JAX_PLATFORMS", "cpu")
import jax
import jax.numpy as jnp

def _softmax(x, axis=-1):
    return jax.nn.softmax(x, axis=axis)
def _gelu(x):
    return jax.nn.gelu(x, approximate=True)
def _silu(x):
    return jax.nn.silu(x)
def _sigmoid(x):
    return jax.nn.sigmoid(x)
def _layernorm(x, axis=-1, eps=1e-5):
    m = jnp.mean(x, axis=axis, keepdims=True)
    v = jnp.var(x, axis=axis, keepdims=True)
    return (x - m) / jnp.sqrt(v + eps)
def _scatter_add(tgt, idx, src, axis=0):
    return tgt.at[idx].add(src)
def _segment_sum(src, seg, n):
    return jax.ops.segment_sum(src, seg, n)
class _Rng:
    def __init__(self, key):
        self._k = key
    def _next(self):
        self._k, sub = jax.random.split(self._k)
        return sub
    def normal(self, shape):
        return jax.random.normal(self._next(), shape, dtype=jnp.bfloat16)
    def randint(self, lo, hi, shape):
        return jax.random.randint(self._next(), shape, lo, hi, dtype=jnp.int32)
    def uniform(self, shape, lo=0.0, hi=1.0):
        return jax.random.uniform(self._next(), shape, jnp.bfloat16, lo, hi)
    def permutation(self, n):
        return jax.random.permutation(self._next(), n)


kernel_name = 'gated_mix__grouped_kv_mqa__swiglu_ffn__prompt'

def setup_inputs():
    _rng = _Rng(jax.random.key(int.from_bytes(__import__("os").urandom(4), "little")))
    _w = (lambda a: (lambda t: t.astype(jnp.bfloat16) if jnp.issubdtype(t.dtype, jnp.floating) else t)(jnp.asarray(a)))
    def _A_setup():
        B, S, D, H = 1, 2048, 512, 32
        Dh = D // H
        return {
            "x": _w((lambda *s: _rng.normal(s) * 0.05)(B, S, D)),
            "wq": _w((lambda *s: _rng.normal(s) * 0.4)(D, H * Dh)),
            "wk": _w((lambda *s: _rng.normal(s) * 0.4)(D, Dh)),
            "wv": _w((lambda *s: _rng.normal(s) * 0.05)(D, Dh)),
            "wo": _w((lambda *s: _rng.normal(s) * 0.05)(H * Dh, D)),
        }
    _A_in = _A_setup()

    def _B_setup():
        B, S, D, F = 1, 2048, 512, 1792
        return {
            "x": _w((lambda *s: _rng.normal(s) * 0.05)(B, S, D)),
            "w_gate": _w((lambda *s: _rng.normal(s) * 0.05)(D, F)),
            "w_up": _w((lambda *s: _rng.normal(s) * 0.05)(D, F)),
            "w_down": _w((lambda *s: _rng.normal(s) * 0.05)(F, D)),
        }
    _B_in = _B_setup()

    return {
        "A_x": _A_in["x"],
        "A_wq": _A_in["wq"],
        "A_wk": _A_in["wk"],
        "A_wv": _A_in["wv"],
        "A_wo": _A_in["wo"],
        "B_x": _B_in["x"],
        "B_w_gate": _B_in["w_gate"],
        "B_w_up": _B_in["w_up"],
        "B_w_down": _B_in["w_down"],
        "gate_w": _w((lambda *s: _rng.normal(s) * 0.05)(512) * 16.0),
    }

def reference(A_x, A_wq, A_wk, A_wv, A_wo, B_x, B_w_gate, B_w_up, B_w_down, gate_w):
    def _A_ref(x, wq, wk, wv, wo):
        B, S, D = x.shape
        H = 32
        Dh = D // H
        q = (lambda x, *d: x.transpose(*d))((x @ wq).reshape(B, S, H, Dh), 0, 2, 1, 3)
        k = x @ wk
        v = x @ wv
        scores = jnp.einsum("bhqd,bkd->bhqk", q, k) * (Dh ** -0.5)
        p = _softmax(scores, axis=-1)
        o = jnp.einsum("bhqk,bkd->bhqd", p, v)
        return (lambda x, *d: x.transpose(*d))(o, 0, 2, 1, 3).reshape(B, S, H * Dh) @ wo

    def _B_ref(x, w_gate, w_up, w_down):
        g = _silu(x @ w_gate)
        u = x @ w_up
        return (g * u) @ w_down

    x = A_x
    g = _sigmoid((x * gate_w).sum(-1, keepdims=True))
    a = _A_ref(x, A_wq, A_wk, A_wv, A_wo)
    b = _B_ref(x, B_w_gate, B_w_up, B_w_down)
    return g * a + (1 - g) * b
```

```python
import functools
import jax
import jax.numpy as jnp
import jax.experimental.pallas as pl
import jax.experimental.pallas.tpu as pltpu

S, D, H, DH, F = 2048, 512, 32, 16, 1792
LOG2E = 1.4426950408889634
F32 = jnp.float32
BF16 = jnp.bfloat16
U32 = jnp.uint32
KC = 128
NC = S // KC
NF = F // 128


def _spread(total, n=NC):
    g = total // 16
    return [16 * ((g * (c + 1)) // n - (g * c) // n) for c in range(n)]


def make_kernel(TQ=512, NV=384, NVE=256, NP=4, LAGT=110, GU0=1, DN0=5, FB=1):
    NL = TQ // 128
    NT = S // TQ
    RP = TQ // NP
    nv_loop = _spread(NV)
    nv_edge = _spread(NVE)
    nvmax = [max(a, b) for a, b in zip(nv_loop, nv_edge)]
    off = [sum(nvmax[:c]) for c in range(NC)]
    NKB = max(sum(nvmax), 16)

    def kernel(x_hbm, wq_hbm, wk_ref, wv_ref, wo_hbm, wg_hbm, wu_hbm, wd_hbm, gw_ref,
               o_ref,
               x_scr, wq_scr, wo_scr, wgu_scr, wd_scr, xp_scr, k_scr, vt_scr, qt_scr, qf_scr,
               kb_scr, p_scr, ot_scr, b_scr, gb_scr, s_scr, sems):
        i = pl.program_id(0)

        def x_copy(c):
            return pltpu.make_async_copy(x_hbm.at[pl.ds(c * TQ, TQ)], x_scr.at[pl.ds(c * TQ, TQ)],
                                         sems.at[c])

        def wq_copy():
            return pltpu.make_async_copy(wq_hbm, wq_scr, sems.at[NT])

        def wo_copy():
            return pltpu.make_async_copy(wo_hbm, wo_scr, sems.at[NT + 1])

        def ffn_copies(j):
            sem = sems.at[NT + 2 + j]
            if isinstance(j, int):
                col = pl.ds(j * 128, 128)
            else:
                col = pl.ds(pl.multiple_of(j * 128, 128), 128)
            return [
                pltpu.make_async_copy(wg_hbm.at[:, col], wgu_scr.at[j, :, pl.ds(0, 128)], sem),
                pltpu.make_async_copy(wu_hbm.at[:, col], wgu_scr.at[j, :, pl.ds(128, 128)], sem),
                pltpu.make_async_copy(wd_hbm.at[col, :], wd_scr.at[j], sem),
            ]

        @pl.when(i == 0)
        def _():
            for c in range(NT):
                x_copy(c).start()
            wq_copy().start()
            r = jax.lax.broadcasted_iota(jnp.int32, (DH, DH * 128), 0)
            cidx = jax.lax.broadcasted_iota(jnp.int32, (DH, DH * 128), 1)
            e = jnp.where(cidx // 128 == r, 1.0, 0.0).astype(BF16)
            for t in range(NT):
                x_copy(t).wait()
                if t == NT - 1:
                    for j in range(NF):
                        for cp in ffn_copies(j):
                            cp.start()
                    wo_copy().start()
                x = x_scr[t * TQ:(t + 1) * TQ, :]
                k = jnp.dot(x, wk_ref[...], preferred_element_type=F32).astype(BF16)
                k_scr[t * TQ // 2:(t + 1) * TQ // 2, :] = pltpu.bitcast(k, U32)
                vt = jax.lax.dot_general(wv_ref[...], x, (((0,), (1,)), ((), ())),
                                         preferred_element_type=F32)
                vt_scr[:, t * TQ:(t + 1) * TQ] = pltpu.bitcast(vt.astype(BF16), U32)
                cs = [c for c in range(t * TQ // KC, (t + 1) * TQ // KC) if nvmax[c]]
                if cs:
                    kv = jnp.concatenate(
                        [k[(c + 1) * KC - nvmax[c] - t * TQ:(c + 1) * KC - t * TQ] for c in cs], axis=0)
                    kb_scr[0, off[cs[0]]:off[cs[-1]] + nvmax[cs[-1]], :] = jnp.dot(
                        kv, e, preferred_element_type=F32)
            wq_copy().wait()

        xt = x_scr[pl.ds(pl.multiple_of(i * TQ, TQ), TQ), :]
        xp_scr[...] = pltpu.bitcast(xt, U32)
        qt = jax.lax.dot_general(wq_scr[...], xt, (((0,), (1,)), ((), ())),
                                 preferred_element_type=F32)
        qt = (qt * (DH ** -0.5 * LOG2E)).astype(BF16)
        qt_scr[...] = pltpu.bitcast(qt, U32).reshape(H, DH // 2, TQ)
        qf_scr[...] = qt.astype(F32).reshape(H, DH, TQ)
        gl = jnp.sum(xt.astype(F32) * gw_ref[...].astype(F32), axis=-1, keepdims=True)
        gb_scr[...] = jnp.broadcast_to(1.0 - jax.nn.sigmoid(gl), (TQ, 128))
        b_scr[...] = jnp.zeros((TQ, D), F32)

        always = jax.lax.broadcasted_iota(jnp.int32, (8, 128), 1) >= (i >> 8)

        def opaque0(h, k):
            return (jnp.asarray(h, jnp.int32) + i) >> (8 + k)

        def a_mxu(c, n, qt_h, l8):
            k0 = c * KC
            kk = pltpu.bitcast(k_scr[k0 // 2:(k0 + n) // 2, :], BF16)
            s = jnp.dot(kk, qt_h, preferred_element_type=F32)
            p = jnp.exp2(s)
            p_scr[k0 // 2:(k0 + n) // 2, :] = pltpu.bitcast(p.astype(BF16), U32)
            ps = p.reshape(n // 8, 8, TQ).sum(axis=0)
            return [l8[j] + ps[:, j * 128:(j + 1) * 128] for j in range(NL)], p

        def a_vpu(c, g0, nvc, j, h, l8j, uid, src):
            z = opaque0(h, uid % 4)
            hq = jnp.asarray(h, jnp.int32) + opaque0(h, 4 + uid % 19)
            r0 = off[c] + nvmax[c] - nvc + g0 * 16
            s = None
            for d in range(DH):
                kb = kb_scr[z, r0:r0 + 16, d * 128:(d + 1) * 128]
                qb = qf_scr[hq, d:d + 1, j * 128:(j + 1) * 128]
                if d == 0 and src is not None:
                    qb = jnp.where(always, jnp.broadcast_to(qb, (8, 128)), src)
                    qb = jnp.concatenate([qb, qb], axis=0)
                t = kb * qb
                s = t if s is None else s + t
            k0 = (c + 1) * KC - nvc + g0 * 16
            p = jnp.exp2(s)
            p_scr[k0 // 2:k0 // 2 + 8, j * 128:(j + 1) * 128] = pltpu.bitcast(p.astype(BF16), U32)
            return l8j + (p[0:8] + p[8:16])

        def c_chunk(c, acc):
            p = pltpu.bitcast(p_scr[c * KC // 2:(c + 1) * KC // 2, :], BF16)
            vt = pltpu.bitcast(vt_scr[:, c * KC:(c + 1) * KC], BF16)
            return acc + jnp.dot(vt, p, preferred_element_type=F32)

        def finish(h, l8, acc, chk):
            l = jnp.sum(l8, axis=0, keepdims=True)
            o = acc * (1.0 / l)
            ot_scr[h] = pltpu.bitcast(o.astype(BF16), U32)
            lo, hi = chk
            oa = jnp.abs(o)
            oa = jnp.maximum(oa[0:8], oa[8:16]) * (2.0 ** -64)
            return jnp.minimum(lo, l8), jnp.maximum(jnp.maximum(hi, l8), oa)

        def ffn_gu(j, r):
            xr = pltpu.bitcast(xp_scr[r * RP // 2:(r + 1) * RP // 2, :], BF16)
            gu = jnp.dot(xr, wgu_scr[j + opaque0(j, r)], preferred_element_type=F32)
            hg = 0.5 * gu[:, :128]
            act = (hg + hg * jnp.tanh(hg)) * (gu[:, 128:] * gb_scr[r * RP:(r + 1) * RP, :])
            return act.astype(BF16), gu

        def ffn_dn(j, r, act):
            dn = jnp.dot(act, wd_scr[j + opaque0(j, r)], preferred_element_type=F32)
            b_scr[r * RP:(r + 1) * RP, :] += dn
            return dn

        z16 = jnp.zeros((DH, TQ), F32)

        def block(stages, nv, l8_in, chk, fj=None):
            ns = len(stages)
            units = []
            for u, (h_a, h_c) in enumerate(stages):
                for c in range(NC):
                    if h_c is not None:
                        units.append(("pv", u, c, 16))
                    units.append(("qk", u, c, KC - nv[c]))
                    if fj is not None:
                        pos = u * NC + c
                        per = ns * NC // NP
                        if pos % per == GU0:
                            units.append(("gu", pos // per, None, 2 * RP))
                        if pos % per == DN0:
                            units.append(("dn", pos // per, None, RP))
                units.append(("fin", u, None, 0))
            T = sum(un[3] for un in units)
            subs = [(u, c, g0, j) for u in range(ns) for c in range(NC)
                    for g0 in range(nv[c] // 16) for j in range(NL)]
            K = len(subs)
            srcs = []
            t = 0
            si = 0
            l8 = [[jnp.zeros((8, 128), F32) for _ in range(NL)] for _ in range(ns)]
            l8_prev = l8_in
            accs = [z16] * ns
            acts = {}
            seen = set()
            qts = [pltpu.bitcast(qt_scr[h_a], BF16) for h_a, _ in stages]

            def add_srcs(v, t0, dur):
                R, L = v.shape[0] // 8, v.shape[1] // 128
                for r in range(R):
                    srcs.append((t0 + dur * (r + 1) / R, v[r * 8:(r + 1) * 8, (r % L) * 128:(r % L + 1) * 128]))

            def flush(force_u=None):
                nonlocal si
                while si < K:
                    u, c, g0, j = subs[si]
                    tau = (si + 0.5) * T / K - LAGT
                    if force_u is None or u > force_u:
                        if (u, c) not in seen or (srcs and tau > srcs[-1][0]) or (not srcs and tau > 0):
                            break
                    cand = [v for (tt, v) in srcs if tt <= tau]
                    src = cand[-1] if cand else None
                    l8[u][j] = a_vpu(c, g0, nv[c], j, stages[u][0], l8[u][j], si, src)
                    si += 1

            for kind, a, b, dur in units:
                if kind == "pv":
                    accs[a] = c_chunk(b, accs[a])
                    seen.add((a, b))
                elif kind == "qk":
                    seen.add((a, b))
                    l8[a], p = a_mxu(b, dur, qts[a], l8[a])
                    add_srcs(p, t, dur)
                elif kind == "gu":
                    acts[a], gu = ffn_gu(fj, a)
                    add_srcs(jnp.concatenate([gu[:, :128], gu[:, 128:]], axis=0), t, dur)
                elif kind == "dn":
                    dn = ffn_dn(fj, a, acts[a])
                    add_srcs(dn, t, dur)
                elif kind == "fin":
                    flush(force_u=a)
                    if stages[a][1] is not None:
                        chk = finish(stages[a][1], l8_prev, accs[a], chk)
                    l8_prev = jnp.concatenate(l8[a], axis=1)
                t += dur
                flush()
            return l8_prev, chk

        chk = (jnp.full((8, TQ), 1.0, F32), jnp.full((8, TQ), 1.0, F32))
        l8, chk = block([(0, None)], nv_edge, None, chk)

        def body(j, carry):
            l8, lo, hi = carry

            @pl.when(i == 0)
            def _():
                for cp in ffn_copies(j):
                    cp.wait()

            h = 2 * j
            l8, (lo, hi) = block([(h + 1, h), (h + 2, h + 1)], nv_loop, l8, (lo, hi), fj=j)
            return l8, lo, hi

        l8, lo, hi = jax.lax.fori_loop(0, NF, body, (l8,) + chk)

        @pl.when(i == 0)
        def _():
            wo_copy().wait()

        h0 = 2 * NF
        l8, chk = block([(h + 1, h) for h in range(h0, H - 1)], nv_edge, l8, (lo, hi))

        def out_proj(lo_h, hi_h):
            ot = pltpu.bitcast(ot_scr[lo_h:hi_h].reshape((hi_h - lo_h) * DH // 2, TQ), BF16)
            return jax.lax.dot_general(ot, wo_scr[lo_h * DH:hi_h * DH, :], (((0,), (0,)), ((), ())),
                                       preferred_element_type=F32)

        acc = z16
        a = None
        for c in range(NC):
            acc = c_chunk(c, acc)
            if c in (1, 6, 11):
                g = c // 5
                pa = out_proj(8 * g, 8 * g + 8)
                a = pa if a is None else a + pa
        lo, hi = finish(H - 1, l8, acc, chk)
        a = a + out_proj(24, 32)

        def combine(a):
            gate = 1.0 - gb_scr[...]
            gate = jnp.concatenate([gate] * (D // 128), axis=1)
            o_ref[...] = (gate * a + b_scr[...]).astype(o_ref.dtype)

        combine(a)

        if FB:
            ok = jnp.logical_and(lo >= 2.0 ** -64, hi <= 2.0 ** 60)
            nbad = jnp.sum(jnp.where(ok, 0.0, 1.0))

            @pl.when(nbad > 0.0)
            def _():
                def head(h, carry):
                    qt_h = pltpu.bitcast(qt_scr[h], BF16)

                    def pass1(c, m8):
                        r0 = pl.multiple_of(c * (KC // 2), KC // 2)
                        kk = pltpu.bitcast(k_scr[pl.ds(r0, KC // 2), :], BF16)
                        s = jnp.dot(kk, qt_h, preferred_element_type=F32)
                        s_scr[c] = s
                        return jnp.maximum(m8, s.reshape(KC // 8, 8, TQ).max(axis=0))

                    m8 = jax.lax.fori_loop(0, NC, pass1, jnp.full((8, TQ), -jnp.inf, F32))
                    m = jnp.max(m8, axis=0, keepdims=True)

                    def pass2(c, cr):
                        l8, acc = cr
                        p = jnp.exp2(s_scr[c] - m)
                        vt = pltpu.bitcast(vt_scr[:, pl.ds(pl.multiple_of(c * KC, KC), KC)], BF16)
                        acc = acc + jnp.dot(vt, p.astype(BF16), preferred_element_type=F32)
                        return l8 + p.reshape(KC // 8, 8, TQ).sum(axis=0), acc

                    l8, acc = jax.lax.fori_loop(0, NC, pass2, (jnp.zeros((8, TQ), F32), z16))
                    l = jnp.sum(l8, axis=0, keepdims=True)
                    ot_scr[h] = pltpu.bitcast((acc * (1.0 / l)).astype(BF16), U32)
                    return carry

                jax.lax.fori_loop(0, H, head, 0)
                combine(out_proj(0, H))

    def full(shape):
        return pl.BlockSpec(shape, lambda i: (0,) * len(shape))

    hbm = pl.BlockSpec(memory_space=pl.ANY)
    call = pl.pallas_call(
        kernel,
        grid=(NT,),
        in_specs=[hbm, hbm, full((D, DH)), full((D, DH)), hbm, hbm, hbm, hbm, full((1, D))],
        out_specs=pl.BlockSpec((TQ, D), lambda i: (i, 0)),
        out_shape=jax.ShapeDtypeStruct((S, D), BF16),
        scratch_shapes=[
            pltpu.VMEM((S, D), BF16),
            pltpu.VMEM((D, D), BF16),
            pltpu.VMEM((D, D), BF16),
            pltpu.VMEM((NF, D, 256), BF16),
            pltpu.VMEM((NF, 128, D), BF16),
            pltpu.VMEM((TQ // 2, D), U32),
            pltpu.VMEM((S // 2, DH), U32),
            pltpu.VMEM((DH // 2, S), U32),
            pltpu.VMEM((H, DH // 2, TQ), U32),
            pltpu.VMEM((H, DH, TQ), F32),
            pltpu.VMEM((2, NKB, DH * 128), F32),
            pltpu.VMEM((S // 2, TQ), U32),
            pltpu.VMEM((H, DH // 2, TQ), U32),
            pltpu.VMEM((TQ, D), F32),
            pltpu.VMEM((TQ, 128), F32),
            pltpu.VMEM((NC, KC, TQ), F32),
            pltpu.SemaphoreType.DMA((NT + 2 + NF,)),
        ],
        compiler_params=pltpu.CompilerParams(
            dimension_semantics=("arbitrary",),
            vmem_limit_bytes=100 * 1024 * 1024),
        name="gmix",
    )

    @jax.jit
    def fn(A_x, A_wq, A_wk, A_wv, A_wo, B_x, B_w_gate, B_w_up, B_w_down, gate_w):
        out = call(A_x.reshape(S, D), A_wq, A_wk, A_wv, A_wo, B_w_gate, B_w_up, B_w_down,
                   gate_w.reshape(1, D))
        return out.reshape(1, S, D)
    return fn


_impl = make_kernel(NV=336)


@jax.jit
def pallas_gated_mix__grouped_kv_mqa__swiglu_ffn__prompt_kernel(
    A_x, A_wq, A_wk, A_wv, A_wo, B_x, B_w_gate, B_w_up, B_w_down, gate_w):
    return _impl(A_x, A_wq, A_wk, A_wv, A_wo, B_x, B_w_gate, B_w_up, B_w_down, gate_w)
```

```python
import jax
import jax.numpy as jnp
import jax.experimental.pallas as pl
import jax.experimental.pallas.tpu as pltpu

S, D, H, DH, F = 2048, 512, 32, 16, 1792
F32, BF16, U32 = jnp.float32, jnp.bfloat16, jnp.uint32
QSCALE = DH ** -0.5 * 1.4426950408889634

TQ = 512
NT = S // TQ
NL = TQ // 128
KC = 128
NC = S // KC
NF = F // 128
L = 4
RP = TQ // 2
KX = 8


def _spread(total, ph):
    g = total // 16
    return [16 * ((g * (c + 1) + ph) // NC - (g * c + ph) // NC) for c in range(NC)]


NV_LOOP, NV_MID, NV_FIRST = _spread(368, 10), _spread(352, 8), _spread(256, 0)
NV_MAX = [max(t) for t in zip(NV_LOOP, NV_MID, NV_FIRST)]
KB_OFF = [sum(NV_MAX[:c]) for c in range(NC)]
NKB = sum(NV_MAX)
_W = dict(qk=80, gu=105, dn=105, pv=120, qp=90, op=90, qm=90, fin=0, lst=0)
CFG_LOOP = dict(nv=NV_LOOP, wt=_W, lag=110, tr=2, pv2=False)
CFG_MID = dict(nv=NV_MID, wt=dict(_W, qk=92, pv=70), lag=90, tr=4, pv2=True)
CFG_FIRST = dict(nv=NV_FIRST, wt=_W, lag=110, tr=1, pv2=False)
CFG_LAST = dict(nv=NV_MID, wt=_W, lag=110, tr=1, pv2=False)

SEM_WQ, SEM_WO, SEM_FFN = NT, NT + 1, NT + 2
SEM_SMALL, SEM_OUT = NT + 2 + NF, NT + 3 + NF


def _place(units, lo, hi):
    fl = {}
    for k, un in enumerate(units):
        fl.setdefault(lo + (k * (hi - lo)) // len(units), []).append(un)
    return fl


def _place_weighted(units, lo, hi):
    fl, acc, tot = {}, 0, sum(u[2] for u in units)
    for un in units:
        fl.setdefault(lo + (acc * (hi - lo)) // tot, []).append(un)
        acc += un[2]
    return fl


def _merge(*lists):
    tagged = [((k + 0.5) / len(l), n, x) for n, l in enumerate(lists) for k, x in enumerate(l)]
    return [x for _, _, x in sorted(tagged, key=lambda z: z[:2])]


def _kernel(x_hbm, wq_hbm, wk_hbm, wv_hbm, wo_hbm, wg_hbm, wu_hbm, wd_hbm, gw_hbm,
            o_hbm,
            x_scr, wq_scr, wqt_scr, wo_scr, wgu_scr, wd_scr, xp_scr, k_scr, vt_scr, qt_scr, qf_scr,
            kb_scr, l_scr, chk_scr, ot_scr, b_scr, gb_scr, s_scr, sems, p0_scr, p1_scr, p2_scr,
            p3_scr, qnxt_scr, qfb_scr, a_scr, o_scr, wkv_scr, gw_scr, flag_ref):
    i = pl.program_id(0)
    par = i & 1
    p_scr = (p0_scr, p1_scr, p2_scr, p3_scr)

    always = jax.lax.broadcasted_iota(jnp.int32, (8, 128), 1) >= (i >> 8)

    def opaque0(h, k):
        return (jnp.asarray(h, jnp.int32) + i) >> (8 + k)

    def x_copy(c):
        return pltpu.make_async_copy(x_hbm.at[pl.ds(c * TQ, TQ)], x_scr.at[pl.ds(c * TQ, TQ)],
                                     sems.at[c])

    def wq_copy():
        return pltpu.make_async_copy(wq_hbm, wq_scr, sems.at[SEM_WQ])

    def wo_copy():
        return pltpu.make_async_copy(wo_hbm, wo_scr, sems.at[SEM_WO])

    def small_copies():
        sem = sems.at[SEM_SMALL]
        return [pltpu.make_async_copy(wk_hbm, wkv_scr.at[pl.ds(0, DH)], sem),
                pltpu.make_async_copy(wv_hbm, wkv_scr.at[pl.ds(DH, DH)], sem),
                pltpu.make_async_copy(gw_hbm, gw_scr, sem)]

    def out_copy(r0, n):
        return pltpu.make_async_copy(o_scr.at[pl.ds(r0, n)],
                                     o_hbm.at[pl.ds(pl.multiple_of(i * TQ + r0, 64), n)],
                                     sems.at[SEM_OUT])

    def ffn_copies(j):
        sem = sems.at[SEM_FFN + j]
        if isinstance(j, int):
            col = pl.ds(j * 128, 128)
        else:
            col = pl.ds(pl.multiple_of(j * 128, 128), 128)
        return [
            pltpu.make_async_copy(wg_hbm.at[:, col], wgu_scr.at[j, :, pl.ds(0, 128)], sem),
            pltpu.make_async_copy(wu_hbm.at[:, col], wgu_scr.at[j, :, pl.ds(128, 128)], sem),
            pltpu.make_async_copy(wd_hbm.at[col, :], wd_scr.at[j], sem),
        ]

    def prep(ts):
        wkv = wkv_scr[...]
        gw = gw_scr[...].astype(F32).reshape(1, D)
        ks = {}
        for t in ts:
            x = x_scr[t * TQ:(t + 1) * TQ, :]
            xp_scr[t] = pltpu.bitcast(x, U32)
            kvt = jax.lax.dot_general(wkv, x, (((1,), (1,)), ((), ())), preferred_element_type=F32)
            vt_scr[:, t * TQ:(t + 1) * TQ] = pltpu.bitcast(kvt[DH:].astype(BF16), U32)
            ks[t] = kvt[:DH].T.astype(BF16)
            k_scr[t * TQ // 2:(t + 1) * TQ // 2, :] = pltpu.bitcast(ks[t], U32)
            gl = jnp.sum(x.astype(F32) * gw, axis=-1, keepdims=True)
            gb_scr[t] = jnp.broadcast_to(0.5 - 0.5 * jnp.tanh(0.5 * gl), (TQ, 128))
        r = jax.lax.broadcasted_iota(jnp.int32, (DH, DH * 128), 0)
        cidx = jax.lax.broadcasted_iota(jnp.int32, (DH, DH * 128), 1)
        e = jnp.where(cidx // 128 == r, 1.0, 0.0).astype(BF16)
        cs = list(range(ts[0] * TQ // KC, (ts[-1] + 1) * TQ // KC))
        kv = jnp.concatenate(
            [ks[c * KC // TQ][(c + 1) * KC - NV_MAX[c] - (c * KC // TQ) * TQ:
                              (c + 1) * KC - (c * KC // TQ) * TQ] for c in cs], axis=0)
        r0, r1 = KB_OFF[cs[0]], KB_OFF[cs[-1]] + NV_MAX[cs[-1]]
        nm = DH - KX
        kb_scr[0, r0:r1, 0:nm * 128] = jnp.dot(kv, e[:, 0:nm * 128], preferred_element_type=F32)
        kf = kv.astype(F32)
        for d in range(nm, DH):
            kb_scr[0, r0:r1, d * 128:(d + 1) * 128] = jnp.broadcast_to(kf[:, d:d + 1], (r1 - r0, 128))

    def q_rows(r0, r1, t, jc=None):
        if jc is None:
            xt = pltpu.bitcast(xp_scr[t], BF16)
        else:
            xt = pltpu.bitcast(xp_scr[t, jc * 64:(jc + 1) * 64, :], BF16)
        w = pltpu.bitcast(wqt_scr[r0 // 2:r1 // 2, :], BF16)
        qt = jax.lax.dot_general(w, xt, (((1,), (1,)), ((), ())), preferred_element_type=F32)
        return qt, (qt * QSCALE).astype(BF16)

    def q_proj(g, jc, t, bz):
        h0 = max(8 * g, L)
        nh = 8 * g + 8 - h0
        cols = slice(jc * 128, (jc + 1) * 128)
        qt, qb = q_rows(h0 * DH, (h0 + nh) * DH, t, jc)
        qt_scr[h0:h0 + nh, :, cols] = pltpu.bitcast(qb, U32).reshape(nh, DH // 2, 128)
        qf_scr[h0:h0 + nh, :, cols] = qb.astype(F32).reshape(nh, DH, 128)
        for r in range(4):
            rr = (r * qt.shape[0] // 8) // 4
            zv = jnp.where(always, 0.0, qt[rr * 8:(rr + 1) * 8, :])
            r0 = ((g * 4 + jc) * 4 + r) * (TQ // 64)
            b_scr[bz, r0:r0 + TQ // 64, :] = jnp.tile(zv, (TQ // 64 // 8, D // 128))
        return qt

    def q_store_first(qb, late=None):
        qt_scr[0:L] = pltpu.bitcast(qb, U32).reshape(L, DH // 2, TQ)
        qf = qb.astype(F32)
        if late is not None:
            qf = jnp.where(jnp.tile(always, (L * DH // 8, NL)), qf, jnp.tile(late, (L * DH // 8, NL)))
        qnxt_scr[...] = qf.reshape(L, DH, TQ)

    def op_unit(otr, g, r0, n):
        rows = slice(r0, r0 + n)
        if g not in otr:
            otr[g] = pltpu.bitcast(ot_scr[8 * g:8 * g + 8].reshape(64, TQ), BF16).T
        pa = jnp.dot(otr[g][rows], wo_scr[g * 128:(g + 1) * 128, :], preferred_element_type=F32)
        if g == 0:
            a_scr[rows, :] = pa
        elif g < 3:
            a_scr[rows, :] += pa
        else:
            gate = 1.0 - gb_scr[i, rows, :]
            gate = jnp.concatenate([gate] * (D // 128), axis=1)
            o_scr[rows, :] = (gate * (a_scr[rows, :] + pa) + b_scr[par, rows, :]).astype(BF16)
            out_copy(r0, n).start()
        return pa

    def scores_mxu(b, c, n, qt_h, l8):
        k0 = c * KC
        kk = pltpu.bitcast(k_scr[k0 // 2:(k0 + n) // 2, :], BF16)
        p = jnp.exp2(jnp.dot(kk, qt_h, preferred_element_type=F32))
        p_scr[b][k0 // 2:(k0 + n) // 2, :] = pltpu.bitcast(p.astype(BF16), U32)
        ps = p.reshape(n // 8, 8, TQ).sum(axis=0)
        return [l8[j] + ps[:, j * 128:(j + 1) * 128] for j in range(NL)], p

    def scores_vpu(b, c, g0, nvc, j, qf, l8, uid, src):
        q_ref, h, salt = qf
        z = opaque0(salt, uid % 4)
        hq = jnp.asarray(h, jnp.int32) + opaque0(salt, 4 + uid % 19)
        r0 = KB_OFF[c] + NV_MAX[c] - nvc + g0 * 16
        step = DH // len(src)
        s = None
        for d in range(DH):
            kb = kb_scr[z, r0:r0 + 16, d * 128:(d + 1) * 128]
            qb = q_ref[hq, d:d + 1, j * 128:(j + 1) * 128]
            if d % step == 0 and src[d // step] is not None:
                qb = jnp.where(always, jnp.broadcast_to(qb, (8, 128)), src[d // step])
                qb = jnp.concatenate([qb, qb], axis=0)
            t = kb * qb
            s = t if s is None else s + t
        k0 = (c + 1) * KC - nvc + g0 * 16
        p = jnp.exp2(s)
        p_scr[b][k0 // 2:k0 // 2 + 8, j * 128:(j + 1) * 128] = pltpu.bitcast(p.astype(BF16), U32)
        l8[j] = l8[j] + (p[0:8] + p[8:16])

    def pv_chunk(b, c, acc):
        p = pltpu.bitcast(p_scr[b][c * KC // 2:(c + 1) * KC // 2, :], BF16)
        vt = pltpu.bitcast(vt_scr[:, c * KC:(c + 1) * KC], BF16)
        return acc + jnp.dot(vt, p, preferred_element_type=F32)

    def finish(b, h, acc):
        l8 = l_scr[b]
        l = jnp.sum(l8, axis=0, keepdims=True)
        o = acc * (1.0 / l)
        ot_scr[h] = pltpu.bitcast(o.astype(BF16), U32)
        chk_scr[0] = jnp.minimum(chk_scr[0], l8)
        chk_scr[1] = jnp.maximum(chk_scr[1], l8)
        chk_scr[2] = chk_scr[2] + (o[0:8] + o[8:16]) * 0.0

    def ffn_gu(j, r):
        xr = pltpu.bitcast(xp_scr[i + opaque0(j, 4 + r), r * RP // 2:(r + 1) * RP // 2, :], BF16)
        gu = jnp.dot(xr, wgu_scr[j + opaque0(j, r)], preferred_element_type=F32)
        hg = 0.5 * gu[:, :128]
        gb = gb_scr[i + opaque0(j, 8 + r), r * RP:(r + 1) * RP, :]
        act = (hg + hg * jnp.tanh(hg)) * (gu[:, 128:] * gb)
        return act.astype(BF16), gu

    def ffn_dn(j, r, act):
        dn = jnp.dot(act, wd_scr[j + opaque0(j, r)], preferred_element_type=F32)
        b_scr[par, r * RP:(r + 1) * RP, :] += dn
        return dn

    z16 = jnp.zeros((DH, TQ), F32)

    def block(stages, cfg, fillers, fj=None):
        nv, wt, tr, pv2 = cfg["nv"], cfg["wt"], cfg["tr"], cfg["pv2"]
        ns = len(stages)
        pvs = [(u, c) for u in range(ns) if stages[u][2] is not None for c in range(NC)]
        units, pi = [], 0
        for u, (ha, _, hc) in enumerate(stages):
            for c in range(NC):
                for _ in range(2 if pv2 else 1):
                    if pi < len(pvs):
                        units.append(("pv",) + pvs[pi] + (16,))
                        if pv2 and pvs[pi][1] == NC - 1:
                            units.append(("fin", pvs[pi][0], None, 0))
                        pi += 1
                if ha is not None:
                    units.append(("qk", u, c, KC - nv[c]))
                for kind, arg, dur in fillers.get(u * NC + c, ()):
                    units.append((kind, arg, None, dur))
            if hc is not None and not pv2:
                units.append(("fin", u, None, 0))
            if ha is not None:
                units.append(("lst", u, None, 0))
        for kind, arg, dur in fillers.get(ns * NC, ()):
            units.append((kind, arg, None, dur))
        total = sum(un[3] * wt[un[0]] / 100 for un in units)
        subs = [(u, c, g0, j) for u in range(ns) if stages[u][0] is not None for c in range(NC)
                for g0 in range(nv[c] // 16) for j in range(NL)]
        nsub = len(subs)
        srcs = []
        state = dict(si=0)
        l8 = [[jnp.zeros((8, 128), F32) for _ in range(NL)] for _ in range(ns)]
        accs = [z16] * ns
        acts, qts, otr, seen, minis = {}, {}, {}, set(), []

        def add_srcs(v, t0, dur):
            nr = v.shape[0] // 8
            for r in range(nr):
                srcs.append((t0 + dur * (r + 1) / nr, v, r))

        def src_at(tau):
            cand = [sv for sv in srcs if sv[0] <= tau]
            if not cand:
                return None
            _, v, r = cand[-1]
            lt = r % (v.shape[1] // 128)
            return v[r * 8:(r + 1) * 8, lt * 128:(lt + 1) * 128]

        def flush(force_u=None):
            while state["si"] < nsub:
                si = state["si"]
                u, c, g0, j = subs[si]
                dt = total / nsub
                tau = (si + 0.5) * dt - cfg["lag"]
                if force_u is None or u > force_u:
                    tend = tau + (tr - 1) * dt / tr
                    if (u, c) not in seen or tend > (srcs[-1][0] if srcs else 0):
                        break
                src = [src_at(tau + r * dt / tr) for r in range(tr)]
                scores_vpu(u, c, g0, nv[c], j, stages[u][1], l8[u], si, src)
                state["si"] = si + 1

        t = 0
        for kind, a, b, n in units:
            dur = n * wt[kind] / 100
            if kind == "pv":
                accs[a] = pv_chunk(a, b, accs[a])
                seen.add((a, b))
            elif kind == "qk":
                seen.add((a, b))
                if a not in qts:
                    qts[a] = pltpu.bitcast(qt_scr[stages[a][0]], BF16)
                l8[a], p = scores_mxu(a, b, n, qts[a], l8[a])
                add_srcs(p, t, dur)
            elif kind == "gu":
                acts[a], gu = ffn_gu(fj[a[0]], a[1])
                add_srcs(gu[:, :128], t, dur / 2)
                add_srcs(gu[:, 128:], t + dur / 2, dur / 2)
            elif kind == "dn":
                add_srcs(ffn_dn(fj[a[0]], a[1], acts[a]), t, dur)
            elif kind == "qp":
                add_srcs(q_proj(*a), t, dur)
            elif kind == "qm":
                qt, qb = q_rows(0, L * DH, a[1], a[0])
                minis.append(qb)
                add_srcs(qt, t, dur)
            elif kind == "op":
                add_srcs(op_unit(otr, *a), t, dur)
            elif kind == "fin":
                hc = stages[a][2]
                finish(a, hc, accs[a])
                if isinstance(hc, int) and hc == H - 1:
                    ok = jnp.logical_and(
                        jnp.logical_and(chk_scr[0] >= 2.0 ** -64, chk_scr[1] <= 2.0 ** 60),
                        chk_scr[2] == 1.0)
                    flag_ref[0] = jnp.sum(jnp.where(ok, 0.0, 1.0))
                    chk_scr[0:3] = jnp.ones((3, 8, TQ), F32)
            elif kind == "lst":
                flush(force_u=a)
                l_scr[a] = jnp.concatenate(l8[a], axis=1)
            t += dur
            flush()
        if minis:
            q_store_first(jnp.concatenate(minis, axis=1), l8[-1][NL - 1])

    @pl.when(i == 0)
    def _():
        for cp in small_copies():
            cp.start()
        x_copy(0).start()
        wq_copy().start()
        for c in range(1, NT):
            x_copy(c).start()
        for cp in small_copies():
            cp.wait()
        x_copy(0).wait()
        prep([0])
        wq_copy().wait()
        wqt_scr[...] = pltpu.bitcast(wq_scr[...].T, U32)
        q_store_first(q_rows(0, L * DH, 0)[1])
        for g in range(4):
            for jc in range(NL):
                q_proj(g, jc, 0, 0)
        for t in range(1, NT):
            x_copy(t).wait()
        for j in range(NF):
            for cp in ffn_copies(j):
                cp.start()
        wo_copy().start()
        prep(list(range(1, NT)))
        chk_scr[0:3] = jnp.ones((3, 8, TQ), F32)

    @pl.when(i < 1)
    def _():
        block([(h, (qnxt_scr, h, h), None) for h in range(L)], CFG_FIRST,
              _place([("qm", (jc, 1), 64) for jc in range(NL)], 1, 63))

    def body(jj, carry):
        js = [2 * jj, 2 * jj + 1]

        @pl.when(i == 0)
        def _():
            for j in js:
                for cp in ffn_copies(j):
                    cp.wait()

        fl = {}
        for a in range(4):
            fl[a * NC + 4] = [("gu", (a // 2, a % 2), 2 * RP)]
            fl[a * NC + 14] = [("dn", (a // 2, a % 2), RP)]
        h = L * jj
        block([(h + u + L, (qf_scr, h + u + L, h + u + L), h + u) for u in range(L)],
              CFG_LOOP, fl, fj=js)
        return carry

    jax.lax.fori_loop(0, NF // 2, body, 0)

    @pl.when(i == 0)
    def _():
        wo_copy().wait()

    @pl.when(i > 0)
    def _():
        out_copy(0, TQ).wait()

    @pl.when(i < NT - 1)
    def _():
        nx = (i + 1, 1 - par)
        qp = [("qp", (g, jc) + nx, 64 if g == 0 else 128) for g in range(4) for jc in range(NL)]
        op = [("op", (g, r, 128), 128) for g in range(4) for r in range(0, TQ, 128)]
        qm = [("qm", (jc, jnp.minimum(i + 2, NT - 1)), 64) for jc in range(NL)]
        fl = _place_weighted(op[:12], 1, 33)
        fl.update(_place_weighted(_merge(qp, qm, op[12:]), 33, 63))
        block([(u, (qnxt_scr, u, H + u), H - L + u) for u in range(L)], CFG_MID, fl)

    @pl.when(i == NT - 1)
    def _():
        op = [("op", (g, r, 64), 64) for g in range(4) for r in range(0, TQ, 64)]
        fl = _place(op[:24], 5, 64)
        fl[64] = op[24:]
        block([(None, None, H - L + u) for u in range(L)], CFG_LAST, fl)

    @pl.when(flag_ref[0] > 0.0)
    def _():
        qfb_scr[...] = pltpu.bitcast(q_rows(0, D, i)[1], U32).reshape(H, DH // 2, TQ)

        def head(h, carry):
            qt_h = pltpu.bitcast(qfb_scr[h], BF16)

            def pass1(c, m8):
                r0 = pl.multiple_of(c * (KC // 2), KC // 2)
                kk = pltpu.bitcast(k_scr[pl.ds(r0, KC // 2), :], BF16)
                s = jnp.dot(kk, qt_h, preferred_element_type=F32)
                s_scr[c] = s
                return jnp.maximum(m8, s.reshape(KC // 8, 8, TQ).max(axis=0))

            m8 = jax.lax.fori_loop(0, NC, pass1, jnp.full((8, TQ), -jnp.inf, F32))
            m = jnp.max(m8, axis=0, keepdims=True)

            def pass2(c, cr):
                l8, acc = cr
                p = jnp.exp2(s_scr[c] - m)
                vt = pltpu.bitcast(vt_scr[:, pl.ds(pl.multiple_of(c * KC, KC), KC)], BF16)
                acc = acc + jnp.dot(vt, p.astype(BF16), preferred_element_type=F32)
                return l8 + p.reshape(KC // 8, 8, TQ).sum(axis=0), acc

            l8, acc = jax.lax.fori_loop(0, NC, pass2, (jnp.zeros((8, TQ), F32), z16))
            l = jnp.sum(l8, axis=0, keepdims=True)
            ot_scr[h] = pltpu.bitcast((acc * (1.0 / l)).astype(BF16), U32)
            return carry

        jax.lax.fori_loop(0, H, head, 0)
        out_copy(0, TQ).wait()
        ot = pltpu.bitcast(ot_scr[...].reshape(D // 2, TQ), BF16)
        a = jax.lax.dot_general(ot, wo_scr[...], (((0,), (0,)), ((), ())),
                                preferred_element_type=F32)
        gate = 1.0 - gb_scr[i]
        gate = jnp.concatenate([gate] * (D // 128), axis=1)
        o_scr[...] = (gate * a + b_scr[par]).astype(BF16)
        out_copy(0, TQ).start()

    @pl.when(i == NT - 1)
    def _():
        out_copy(0, TQ).wait()


@jax.jit
def pallas_gated_mix__grouped_kv_mqa__swiglu_ffn__prompt_kernel(
    A_x: jax.Array,
    A_wq: jax.Array,
    A_wk: jax.Array,
    A_wv: jax.Array,
    A_wo: jax.Array,
    B_x: jax.Array,
    B_w_gate: jax.Array,
    B_w_up: jax.Array,
    B_w_down: jax.Array,
    gate_w: jax.Array,
):
    del B_x
    hbm = pl.BlockSpec(memory_space=pl.ANY)
    out = pl.pallas_call(
        _kernel,
        grid=(NT,),
        in_specs=[hbm] * 9,
        out_specs=hbm,
        out_shape=jax.ShapeDtypeStruct((S, D), BF16),
        scratch_shapes=[
            pltpu.VMEM((S, D), BF16),
            pltpu.VMEM((D, D), BF16),
            pltpu.VMEM((D // 2, D), U32),
            pltpu.VMEM((D, D), BF16),
            pltpu.VMEM((NF, D, 256), BF16),
            pltpu.VMEM((NF, 128, D), BF16),
            pltpu.VMEM((NT, TQ // 2, D), U32),
            pltpu.VMEM((S // 2, DH), U32),
            pltpu.VMEM((DH // 2, S), U32),
            pltpu.VMEM((H, DH // 2, TQ), U32),
            pltpu.VMEM((H, DH, TQ), F32),
            pltpu.VMEM((2, NKB, DH * 128), F32),
            pltpu.VMEM((L, 8, TQ), F32),
            pltpu.VMEM((4, 8, TQ), F32),
            pltpu.VMEM((H, DH // 2, TQ), U32),
            pltpu.VMEM((2, TQ, D), F32),
            pltpu.VMEM((NT, TQ, 128), F32),
            pltpu.VMEM((NC, KC, TQ), F32),
            pltpu.SemaphoreType.DMA((NT + 4 + NF,)),
            pltpu.VMEM((S // 2, TQ), U32),
            pltpu.VMEM((S // 2, TQ), U32),
            pltpu.VMEM((S // 2, TQ), U32),
            pltpu.VMEM((S // 2, TQ), U32),
            pltpu.VMEM((L, DH, TQ), F32),
            pltpu.VMEM((H, DH // 2, TQ), U32),
            pltpu.VMEM((TQ, D), F32),
            pltpu.VMEM((TQ, D), BF16),
            pltpu.VMEM((2 * DH, D), BF16),
            pltpu.VMEM((D,), BF16),
            pltpu.SMEM((1,), F32),
        ],
        compiler_params=pltpu.CompilerParams(
            dimension_semantics=("arbitrary",),
            vmem_limit_bytes=100 * 1024 * 1024),
        name="gmix",
    )(A_x.reshape(S, D), A_wq, A_wk.T, A_wv.T, A_wo, B_w_gate, B_w_up, B_w_down, gate_w)
    return out.reshape(1, S, D)
```

```python
import jax
import jax.numpy as jnp
import jax.experimental.pallas as pl
import jax.experimental.pallas.tpu as pltpu

S, D, H, DH, F = 2048, 512, 32, 16, 1792
F32, BF16, U32 = jnp.float32, jnp.bfloat16, jnp.uint32
QSCALE = DH ** -0.5 * 1.4426950408889634

TQ = 512
NT = S // TQ
NL = TQ // 128
KC = 128
NC = S // KC
NF = F // 128
L = 4
RP = TQ // 2
KX = 8


def _spread(total, ph):
    g = total // 16
    return [16 * ((g * (c + 1) + ph) // NC - (g * c + ph) // NC) for c in range(NC)]


NV_LOOP, NV_MID, NV_FIRST = _spread(368, 10), _spread(352, 8), _spread(256, 0)
NV_MAX = [max(t) for t in zip(NV_LOOP, NV_MID, NV_FIRST)]
KB_OFF = [sum(NV_MAX[:c]) for c in range(NC)]
NKB = sum(NV_MAX)
_W = dict(qk=80, gu=105, dn=105, pv=120, qp=90, op=90, qm=90, fin=0, lst=0, pre=0)
CFG_LOOP = dict(nv=NV_LOOP, wt=_W, lag=110, tr=2, pv2=False,
                shift=(30, 34, 30, 30, 14, 6, 0, 0, 0, 0, 0, 0, 4, 0, 0, -8,
                       0, 0, -2, 12, -6, -6, 0, 12, 0, 0, 12, 10, 6, 6, 13, 45))
CFG_MID = dict(nv=NV_MID, wt=dict(_W, qk=92, pv=80), lag=90, tr=4, pv2=True,
               shift=(20, 30, 45, 6, 45, 0, 0, -12, -30, 0, 0, 0, 6, 6, 0, 0))
CFG_FIRST = dict(nv=NV_FIRST, wt=_W, lag=110, tr=1, pv2=False, shift=(0,))
CFG_LAST = dict(nv=NV_MID, wt=_W, lag=110, tr=1, pv2=False, shift=(0,))

SEM_WQ, SEM_WO, SEM_FFN = NT, NT + 1, NT + 2
SEM_SMALL, SEM_OUT = NT + 2 + NF, NT + 3 + NF


def _place(units, lo, hi):
    fl = {}
    for k, un in enumerate(units):
        fl.setdefault(lo + (k * (hi - lo)) // len(units), []).append(un)
    return fl


def _place_weighted(units, lo, hi):
    fl, acc, tot = {}, 0, sum(u[2] for u in units)
    for un in units:
        fl.setdefault(lo + (acc * (hi - lo)) // tot, []).append(un)
        acc += un[2]
    return fl


def _merge(*lists):
    tagged = [((k + 0.5) / len(l), n, x) for n, l in enumerate(lists) for k, x in enumerate(l)]
    return [x for _, _, x in sorted(tagged, key=lambda z: z[:2])]


def _kernel(x_hbm, wq_hbm, wk_hbm, wv_hbm, wo_hbm, wg_hbm, wu_hbm, wd_hbm, gw_hbm,
            o_hbm,
            x_scr, wq_scr, wqt_scr, wo_scr, wgu_scr, wd_scr, xp_scr, k_scr, vt_scr, qt_scr, qf_scr,
            kb_scr, l_scr, chk_scr, ot_scr, b_scr, gb_scr, s_scr, sems, p0_scr, p1_scr, p2_scr,
            p3_scr, qnxt_scr, qfb_scr, a_scr, o_scr, wkv_scr, gw_scr, flag_ref):
    i = pl.program_id(0)
    par = i & 1
    p_scr = (p0_scr, p1_scr, p2_scr, p3_scr)

    always = jax.lax.broadcasted_iota(jnp.int32, (8, 128), 1) >= (i >> 8)

    def opaque0(h, k):
        return (jnp.asarray(h, jnp.int32) + i) >> (8 + k)

    def x_copy(c):
        return pltpu.make_async_copy(x_hbm.at[pl.ds(c * TQ, TQ)], x_scr.at[pl.ds(c * TQ, TQ)],
                                     sems.at[c])

    def wq_copy():
        return pltpu.make_async_copy(wq_hbm, wq_scr, sems.at[SEM_WQ])

    def wo_copy():
        return pltpu.make_async_copy(wo_hbm, wo_scr, sems.at[SEM_WO])

    def small_copies():
        sem = sems.at[SEM_SMALL]
        return [pltpu.make_async_copy(wk_hbm, wkv_scr.at[pl.ds(0, DH)], sem),
                pltpu.make_async_copy(wv_hbm, wkv_scr.at[pl.ds(DH, DH)], sem),
                pltpu.make_async_copy(gw_hbm, gw_scr, sem)]

    def out_copy(r0, n):
        return pltpu.make_async_copy(o_scr.at[pl.ds(r0, n)],
                                     o_hbm.at[pl.ds(pl.multiple_of(i * TQ + r0, 64), n)],
                                     sems.at[SEM_OUT])

    def ffn_copies(j):
        sem = sems.at[SEM_FFN + j]
        if isinstance(j, int):
            col = pl.ds(j * 128, 128)
        else:
            col = pl.ds(pl.multiple_of(j * 128, 128), 128)
        return [
            pltpu.make_async_copy(wg_hbm.at[:, col], wgu_scr.at[j, :, pl.ds(0, 128)], sem),
            pltpu.make_async_copy(wu_hbm.at[:, col], wgu_scr.at[j, :, pl.ds(128, 128)], sem),
            pltpu.make_async_copy(wd_hbm.at[col, :], wd_scr.at[j], sem),
        ]

    def prep(ts, between=None):
        wkv = wkv_scr[...]
        gw = gw_scr[...].astype(F32).reshape(1, D)
        ks = {}
        for t in ts:
            x = x_scr[t * TQ:(t + 1) * TQ, :]
            xp_scr[t] = pltpu.bitcast(x, U32)
            kvt = jax.lax.dot_general(wkv, x, (((1,), (1,)), ((), ())), preferred_element_type=F32)
            vt_scr[:, t * TQ:(t + 1) * TQ] = pltpu.bitcast(kvt[DH:].astype(BF16), U32)
            ks[t] = kvt[:DH].T.astype(BF16)
            k_scr[t * TQ // 2:(t + 1) * TQ // 2, :] = pltpu.bitcast(ks[t], U32)
            gl = jnp.sum(x.astype(F32) * gw, axis=-1, keepdims=True)
            gb_scr[t] = jnp.broadcast_to(0.5 - 0.5 * jnp.tanh(0.5 * gl), (TQ, 128))
        if between is not None:
            between()
        r = jax.lax.broadcasted_iota(jnp.int32, (DH, DH * 128), 0)
        cidx = jax.lax.broadcasted_iota(jnp.int32, (DH, DH * 128), 1)
        e = jnp.where(cidx // 128 == r, 1.0, 0.0).astype(BF16)
        cs = list(range(ts[0] * TQ // KC, (ts[-1] + 1) * TQ // KC))
        kv = jnp.concatenate(
            [ks[c * KC // TQ][(c + 1) * KC - NV_MAX[c] - (c * KC // TQ) * TQ:
                              (c + 1) * KC - (c * KC // TQ) * TQ] for c in cs], axis=0)
        r0, r1 = KB_OFF[cs[0]], KB_OFF[cs[-1]] + NV_MAX[cs[-1]]
        nm = DH - KX
        kb_scr[0, r0:r1, 0:nm * 128] = jnp.dot(kv, e[:, 0:nm * 128], preferred_element_type=F32)
        kf = kv.astype(F32)
        for d in range(nm, DH):
            kb_scr[0, r0:r1, d * 128:(d + 1) * 128] = jnp.broadcast_to(kf[:, d:d + 1], (r1 - r0, 128))

    def q_rows(r0, r1, t, jc=None):
        if jc is None:
            xt = pltpu.bitcast(xp_scr[t], BF16)
        else:
            xt = pltpu.bitcast(xp_scr[t, jc * 64:(jc + 1) * 64, :], BF16)
        w = pltpu.bitcast(wqt_scr[r0 // 2:r1 // 2, :], BF16)
        qt = jax.lax.dot_general(w, xt, (((1,), (1,)), ((), ())), preferred_element_type=F32)
        return qt, (qt * QSCALE).astype(BF16)

    def q_proj(g, jc, t, bz):
        h0 = max(8 * g, L)
        nh = 8 * g + 8 - h0
        cols = slice(jc * 128, (jc + 1) * 128)
        qt, qb = q_rows(h0 * DH, (h0 + nh) * DH, t, jc)
        qt_scr[h0:h0 + nh, :, cols] = pltpu.bitcast(qb, U32).reshape(nh, DH // 2, 128)
        qf_scr[h0:h0 + nh, :, cols] = qb.astype(F32).reshape(nh, DH, 128)
        for r in range(4):
            rr = (r * qt.shape[0] // 8) // 4
            zv = jnp.where(always, 0.0, qt[rr * 8:(rr + 1) * 8, :])
            r0 = ((g * 4 + jc) * 4 + r) * (TQ // 64)
            b_scr[bz, r0:r0 + TQ // 64, :] = jnp.tile(zv, (TQ // 64 // 8, D // 128))
        return qt

    def q_store_first(qb, late=None):
        qt_scr[0:L] = pltpu.bitcast(qb, U32).reshape(L, DH // 2, TQ)
        qf = qb.astype(F32)
        if late is not None:
            qf = jnp.where(jnp.tile(always, (L * DH // 8, NL)), qf, jnp.tile(late, (L * DH // 8, NL)))
        qnxt_scr[...] = qf.reshape(L, DH, TQ)

    def op_unit(otr, g, r0, n):
        rows = slice(r0, r0 + n)
        if g not in otr:
            otr[g] = pltpu.bitcast(ot_scr[8 * g:8 * g + 8].reshape(64, TQ), BF16).T
        pa = jnp.dot(otr[g][rows], wo_scr[g * 128:(g + 1) * 128, :], preferred_element_type=F32)
        if g == 0:
            a_scr[rows, :] = pa
        elif g < 3:
            a_scr[rows, :] += pa
        else:
            gate = 1.0 - gb_scr[i, rows, :]
            gate = jnp.concatenate([gate] * (D // 128), axis=1)
            o_scr[rows, :] = (gate * (a_scr[rows, :] + pa) + b_scr[par, rows, :]).astype(BF16)
            out_copy(r0, n).start()
        return pa

    def scores_mxu(b, c, n, qt_h, l8):
        k0 = c * KC
        kk = pltpu.bitcast(k_scr[k0 // 2:(k0 + n) // 2, :], BF16)
        p = jnp.exp2(jnp.dot(kk, qt_h, preferred_element_type=F32))
        p_scr[b][k0 // 2:(k0 + n) // 2, :] = pltpu.bitcast(p.astype(BF16), U32)
        ps = p.reshape(n // 8, 8, TQ).sum(axis=0)
        return [l8[j] + ps[:, j * 128:(j + 1) * 128] for j in range(NL)], p

    def scores_vpu(b, c, g0, nvc, j, qf, l8, uid, src):
        q_ref, h, salt = qf
        z = opaque0(salt, uid % 4)
        hq = jnp.asarray(h, jnp.int32) + opaque0(salt, 4 + uid % 19)
        r0 = KB_OFF[c] + NV_MAX[c] - nvc + g0 * 16
        step = DH // len(src)
        s = None
        for d in range(DH):
            kb = kb_scr[z, r0:r0 + 16, d * 128:(d + 1) * 128]
            qb = q_ref[hq, d:d + 1, j * 128:(j + 1) * 128]
            if d % step == 0 and src[d // step] is not None:
                qb = jnp.where(always, jnp.broadcast_to(qb, (8, 128)), src[d // step])
                qb = jnp.concatenate([qb, qb], axis=0)
            t = kb * qb
            s = t if s is None else s + t
        k0 = (c + 1) * KC - nvc + g0 * 16
        p = jnp.exp2(s)
        p_scr[b][k0 // 2:k0 // 2 + 8, j * 128:(j + 1) * 128] = pltpu.bitcast(p.astype(BF16), U32)
        l8[j] = l8[j] + (p[0:8] + p[8:16])

    def p_load(b, c):
        return pltpu.bitcast(p_scr[b][c * KC // 2:(c + 1) * KC // 2, :], BF16)

    def pv_chunk(p, c, acc):
        vt = pltpu.bitcast(vt_scr[:, c * KC:(c + 1) * KC], BF16)
        return acc + jnp.dot(vt, p, preferred_element_type=F32)

    def finish(b, h, acc):
        l8 = l_scr[b]
        l = jnp.sum(l8, axis=0, keepdims=True)
        o = acc * (1.0 / l)
        ot_scr[h] = pltpu.bitcast(o.astype(BF16), U32)
        chk_scr[0] = jnp.minimum(chk_scr[0], l8)
        chk_scr[1] = jnp.maximum(chk_scr[1], l8)
        chk_scr[2] = chk_scr[2] + (o[0:8] + o[8:16]) * 0.0

    def ffn_gu(j, r):
        xr = pltpu.bitcast(xp_scr[i + opaque0(j, 4 + r), r * RP // 2:(r + 1) * RP // 2, :], BF16)
        gu = jnp.dot(xr, wgu_scr[j + opaque0(j, r)], preferred_element_type=F32)
        hg = 0.5 * gu[:, :128]
        gb = gb_scr[i + opaque0(j, 8 + r), r * RP:(r + 1) * RP, :]
        act = (hg + hg * jnp.tanh(hg)) * (gu[:, 128:] * gb)
        return act.astype(BF16), gu

    def ffn_dn(j, r, act):
        dn = jnp.dot(act, wd_scr[j + opaque0(j, r)], preferred_element_type=F32)
        b_scr[par, r * RP:(r + 1) * RP, :] += dn
        return dn

    z16 = jnp.zeros((DH, TQ), F32)

    def block(stages, cfg, fillers, fj=None):
        nv, wt, tr, pv2 = cfg["nv"], cfg["wt"], cfg["tr"], cfg["pv2"]
        ns = len(stages)
        pvs = [(u, c) for u in range(ns) if stages[u][2] is not None for c in range(NC)]
        units, pi = [], 0
        for u, (ha, _, hc) in enumerate(stages):
            for c in range(NC):
                if pv2:
                    if u == 0 and c == 0:
                        units.append(("pre", 0, 0, 0))
                    units.append(("qk", u, c, KC - nv[c]))
                for _ in range(2 if pv2 else 1):
                    if pi < len(pvs):
                        units.append(("pv",) + pvs[pi] + (16,))
                        if pv2 and pvs[pi][1] == NC - 1:
                            units.append(("fin", pvs[pi][0], None, 0))
                        pi += 1
                if ha is not None and not pv2:
                    units.append(("qk", u, c, KC - nv[c]))
                for kind, arg, dur in fillers.get(u * NC + c, ()):
                    units.append((kind, arg, None, dur))
            if hc is not None and not pv2:
                units.append(("fin", u, None, 0))
            if ha is not None:
                units.append(("lst", u, None, 0))
        for kind, arg, dur in fillers.get(ns * NC, ()):
            units.append((kind, arg, None, dur))
        total = sum(un[3] * wt[un[0]] / 100 for un in units)
        subs = [(u, c, g0, j) for u in range(ns) if stages[u][0] is not None for c in range(NC)
                for g0 in range(nv[c] // 16) for j in range(NL)]
        nsub = len(subs)
        srcs = []
        state = dict(si=0)
        l8 = [[jnp.zeros((8, 128), F32) for _ in range(NL)] for _ in range(ns)]
        accs = [z16] * ns
        acts, qts, otr, pre, seen, minis = {}, {}, {}, {}, set(), []

        def add_srcs(v, t0, dur):
            nr = v.shape[0] // 8
            for r in range(nr):
                srcs.append((t0 + dur * (r + 1) / nr, v, r))

        def src_at(tau):
            cand = [sv for sv in srcs if sv[0] <= tau]
            if not cand:
                return None
            _, v, r = cand[-1]
            lt = r % (v.shape[1] // 128)
            return v[r * 8:(r + 1) * 8, lt * 128:(lt + 1) * 128]

        def flush(force_u=None):
            while state["si"] < nsub:
                si = state["si"]
                u, c, g0, j = subs[si]
                dt = total / nsub
                tau = (si + 0.5) * dt - cfg["lag"] + cfg["shift"][si * len(cfg["shift"]) // nsub]
                if force_u is None or u > force_u:
                    tend = tau + (tr - 1) * dt / tr
                    if (u, c) not in seen or tend > (srcs[-1][0] if srcs else 0):
                        break
                src = [src_at(tau + r * dt / tr) for r in range(tr)]
                scores_vpu(u, c, g0, nv[c], j, stages[u][1], l8[u], si, src)
                state["si"] = si + 1

        t = 0
        for kind, a, b, n in units:
            dur = n * wt[kind] / 100
            if kind == "pre":
                pre[(a, b)] = p_load(a, b)
            elif kind == "pv":
                p = pre[(a, b)] if (a, b) in pre else p_load(a, b)
                accs[a] = pv_chunk(p, b, accs[a])
                seen.add((a, b))
            elif kind == "qk":
                seen.add((a, b))
                if a not in qts:
                    qts[a] = pltpu.bitcast(qt_scr[stages[a][0]], BF16)
                l8[a], p = scores_mxu(a, b, n, qts[a], l8[a])
                add_srcs(p, t, dur)
            elif kind == "gu":
                acts[a], gu = ffn_gu(fj[a[0]], a[1])
                add_srcs(gu[:, :128], t, dur / 2)
                add_srcs(gu[:, 128:], t + dur / 2, dur / 2)
            elif kind == "dn":
                add_srcs(ffn_dn(fj[a[0]], a[1], acts[a]), t, dur)
            elif kind == "qp":
                add_srcs(q_proj(*a), t, dur)
            elif kind == "qm":
                qt, qb = q_rows(0, L * DH, a[1], a[0])
                minis.append(qb)
                add_srcs(qt, t, dur)
            elif kind == "op":
                add_srcs(op_unit(otr, *a), t, dur)
            elif kind == "fin":
                hc = stages[a][2]
                finish(a, hc, accs[a])
                if isinstance(hc, int) and hc == H - 1:
                    ok = jnp.logical_and(
                        jnp.logical_and(chk_scr[0] >= 2.0 ** -27, chk_scr[1] <= 2.0 ** 60),
                        chk_scr[2] == 1.0)
                    flag_ref[0] = jnp.sum(jnp.where(ok, 0.0, 1.0))
                    chk_scr[0:3] = jnp.ones((3, 8, TQ), F32)
            elif kind == "lst":
                flush(force_u=a)
                l_scr[a] = jnp.concatenate(l8[a], axis=1)
            t += dur
            flush()
        if minis:
            q_store_first(jnp.concatenate(minis, axis=1), l8[-1][NL - 1])

    @pl.when(i == 0)
    def _():
        for cp in small_copies():
            cp.start()
        x_copy(0).start()
        wq_copy().start()
        for c in range(1, NT):
            x_copy(c).start()
        for cp in small_copies():
            cp.wait()
        x_copy(0).wait()
        prep([0])
        wq_copy().wait()
        wqt_scr[...] = pltpu.bitcast(wq_scr[...].T, U32)
        q_store_first(q_rows(0, L * DH, 0)[1])

        def q_groups(gs):
            for g in gs:
                for jc in range(NL):
                    q_proj(g, jc, 0, 0)

        q_groups([0, 1])
        x_copy(1).wait()
        prep([1], lambda: q_groups([2, 3]))
        x_copy(2).wait()
        x_copy(3).wait()
        for j in range(NF):
            for cp in ffn_copies(j):
                cp.start()
        wo_copy().start()
        prep([2, 3])
        chk_scr[0:3] = jnp.ones((3, 8, TQ), F32)

    @pl.when(i < 1)
    def _():
        block([(h, (qnxt_scr, h, h), None) for h in range(L)], CFG_FIRST,
              _place([("qm", (jc, 1), 64) for jc in range(NL)], 1, 63))

    def body(jj, carry):
        js = [2 * jj, 2 * jj + 1]

        @pl.when(i == 0)
        def _():
            for j in js:
                for cp in ffn_copies(j):
                    cp.wait()

        fl = {}
        for a in range(4):
            fl[a * NC + 4] = [("gu", (a // 2, a % 2), 2 * RP)]
            fl[a * NC + 14] = [("dn", (a // 2, a % 2), RP)]
        h = L * jj
        block([(h + u + L, (qf_scr, h + u + L, h + u + L), h + u) for u in range(L)],
              CFG_LOOP, fl, fj=js)
        return carry

    jax.lax.fori_loop(0, NF // 2, body, 0)

    @pl.when(i == 0)
    def _():
        wo_copy().wait()

    @pl.when(i > 0)
    def _():
        out_copy(0, TQ).wait()

    @pl.when(i < NT - 1)
    def _():
        nx = (i + 1, 1 - par)
        qp = [("qp", (g, jc) + nx, 64 if g == 0 else 128) for g in range(4) for jc in range(NL)]
        op = [("op", (g, r, 128), 128) for g in range(4) for r in range(0, TQ, 128)]
        qm = [("qm", (jc, jnp.minimum(i + 2, NT - 1)), 64) for jc in range(NL)]
        fl = _place_weighted(op[:12], 1, 33)
        fl.update(_place_weighted(_merge(qp, qm, op[12:]), 33, 63))
        block([(u, (qnxt_scr, u, H + u), H - L + u) for u in range(L)], CFG_MID, fl)

    @pl.when(i == NT - 1)
    def _():
        op = [("op", (g, r, 64), 64) for g in range(4) for r in range(0, TQ, 64)]
        fl = _place(op[:24], 5, 64)
        fl[64] = op[24:]
        block([(None, None, H - L + u) for u in range(L)], CFG_LAST, fl)

    @pl.when(flag_ref[0] > 0.0)
    def _():
        qfb_scr[...] = pltpu.bitcast(q_rows(0, D, i)[1], U32).reshape(H, DH // 2, TQ)

        def head(h, carry):
            qt_h = pltpu.bitcast(qfb_scr[h], BF16)

            def pass1(c, m8):
                r0 = pl.multiple_of(c * (KC // 2), KC // 2)
                kk = pltpu.bitcast(k_scr[pl.ds(r0, KC // 2), :], BF16)
                s = jnp.dot(kk, qt_h, preferred_element_type=F32)
                s_scr[c] = s
                return jnp.maximum(m8, s.reshape(KC // 8, 8, TQ).max(axis=0))

            m8 = jax.lax.fori_loop(0, NC, pass1, jnp.full((8, TQ), -jnp.inf, F32))
            m = jnp.max(m8, axis=0, keepdims=True)

            def pass2(c, cr):
                l8, acc = cr
                p = jnp.exp2(s_scr[c] - m)
                vt = pltpu.bitcast(vt_scr[:, pl.ds(pl.multiple_of(c * KC, KC), KC)], BF16)
                acc = acc + jnp.dot(vt, p.astype(BF16), preferred_element_type=F32)
                return l8 + p.reshape(KC // 8, 8, TQ).sum(axis=0), acc

            l8, acc = jax.lax.fori_loop(0, NC, pass2, (jnp.zeros((8, TQ), F32), z16))
            l = jnp.sum(l8, axis=0, keepdims=True)
            ot_scr[h] = pltpu.bitcast((acc * (1.0 / l)).astype(BF16), U32)
            return carry

        jax.lax.fori_loop(0, H, head, 0)
        out_copy(0, TQ).wait()
        ot = pltpu.bitcast(ot_scr[...].reshape(D // 2, TQ), BF16)
        a = jax.lax.dot_general(ot, wo_scr[...], (((0,), (0,)), ((), ())),
                                preferred_element_type=F32)
        gate = 1.0 - gb_scr[i]
        gate = jnp.concatenate([gate] * (D // 128), axis=1)
        o_scr[...] = (gate * a + b_scr[par]).astype(BF16)
        out_copy(0, TQ).start()

    @pl.when(i == NT - 1)
    def _():
        out_copy(0, TQ).wait()


@jax.jit
def pallas_gated_mix__grouped_kv_mqa__swiglu_ffn__prompt_kernel(
    A_x: jax.Array,
    A_wq: jax.Array,
    A_wk: jax.Array,
    A_wv: jax.Array,
    A_wo: jax.Array,
    B_x: jax.Array,
    B_w_gate: jax.Array,
    B_w_up: jax.Array,
    B_w_down: jax.Array,
    gate_w: jax.Array,
):
    del B_x
    hbm = pl.BlockSpec(memory_space=pl.ANY)
    out = pl.pallas_call(
        _kernel,
        grid=(NT,),
        in_specs=[hbm] * 9,
        out_specs=hbm,
        out_shape=jax.ShapeDtypeStruct((S, D), BF16),
        scratch_shapes=[
            pltpu.VMEM((S, D), BF16),
            pltpu.VMEM((D, D), BF16),
            pltpu.VMEM((D // 2, D), U32),
            pltpu.VMEM((D, D), BF16),
            pltpu.VMEM((NF, D, 256), BF16),
            pltpu.VMEM((NF, 128, D), BF16),
            pltpu.VMEM((NT, TQ // 2, D), U32),
            pltpu.VMEM((S // 2, DH), U32),
            pltpu.VMEM((DH // 2, S), U32),
            pltpu.VMEM((H, DH // 2, TQ), U32),
            pltpu.VMEM((H, DH, TQ), F32),
            pltpu.VMEM((2, NKB, DH * 128), F32),
            pltpu.VMEM((L, 8, TQ), F32),
            pltpu.VMEM((4, 8, TQ), F32),
            pltpu.VMEM((H, DH // 2, TQ), U32),
            pltpu.VMEM((2, TQ, D), F32),
            pltpu.VMEM((NT, TQ, 128), F32),
            pltpu.VMEM((NC, KC, TQ), F32),
            pltpu.SemaphoreType.DMA((NT + 4 + NF,)),
            pltpu.VMEM((S // 2, TQ), U32),
            pltpu.VMEM((S // 2, TQ), U32),
            pltpu.VMEM((S // 2, TQ), U32),
            pltpu.VMEM((S // 2, TQ), U32),
            pltpu.VMEM((L, DH, TQ), F32),
            pltpu.VMEM((H, DH // 2, TQ), U32),
            pltpu.VMEM((TQ, D), F32),
            pltpu.VMEM((TQ, D), BF16),
            pltpu.VMEM((2 * DH, D), BF16),
            pltpu.VMEM((D,), BF16),
            pltpu.SMEM((1,), F32),
        ],
        compiler_params=pltpu.CompilerParams(
            dimension_semantics=("arbitrary",),
            vmem_limit_bytes=100 * 1024 * 1024),
        name="gmix",
    )(A_x.reshape(S, D), A_wq, A_wk.T, A_wv.T, A_wo, B_w_gate, B_w_up, B_w_down, gate_w)
    return out.reshape(1, S, D)
```
